```python
import os as _os
_os.environ.setdefault('JAX_PLATFORMS', 'cpu')
import jax
import jax.numpy as jnp

def _softmax(x, axis=-1):
    return jax.nn.softmax(x, axis=axis)

def _gelu(x):
    return jax.nn.gelu(x, approximate=True)

def _silu(x):
    return jax.nn.silu(x)

def _sigmoid(x):
    return jax.nn.sigmoid(x)

def _layernorm(x, axis=-1, eps=1e-05):
    m = jnp.mean(x, axis=axis, keepdims=True)
    v = jnp.var(x, axis=axis, keepdims=True)
    return (x - m) / jnp.sqrt(v + eps)

def _scatter_add(tgt, idx, src, axis=0):
    return tgt.at[idx].add(src)

def _segment_sum(src, seg, n):
    return jax.ops.segment_sum(src, seg, n)

class _Rng:

    def __init__(self, key):
        self._k = key

    def _next(self):
        self._k, sub = jax.random.split(self._k)
        return sub

    def normal(self, shape):
        return jax.random.normal(self._next(), shape, dtype=jnp.bfloat16)

    def randint(self, lo, hi, shape):
        return jax.random.randint(self._next(), shape, lo, hi, dtype=jnp.int32)

    def uniform(self, shape, lo=0.0, hi=1.0):
        return jax.random.uniform(self._next(), shape, jnp.bfloat16, lo, hi)

    def permutation(self, n):
        return jax.random.permutation(self._next(), n)
kernel_name = 'standalone__window_attn_twins__vision'

def setup_inputs():
    _rng = _Rng(jax.random.key(int.from_bytes(__import__("os").urandom(4), "little")))
    _w = lambda a: (lambda t: t.astype(jnp.bfloat16) if jnp.issubdtype(t.dtype, jnp.floating) else t)(jnp.asarray(a))
    H = W = 384 // 8 * 8
    C = 96
    return {'x': _w((lambda *s: _rng.normal(s) * 0.4)(1, H, W, C)), 'wq': _w((lambda *s: _rng.normal(s) * 0.4)(C, C)), 'wkv': _w((lambda *s: _rng.normal(s) * 0.4)(C, 2 * C)), 'wo': _w((lambda *s: _rng.normal(s) * 0.05)(C, C))}

def reference(x, wq, wkv, wo):
    B, H, W, C = x.shape
    win = 8
    nh, nw = (H // win, W // win)
    xs = x.reshape(B, nh, win, nw, win, C).mean(axis=(2, 4)).reshape(B, nh * nw, C)
    q = x.reshape(B, H * W, C) @ wq
    kv = xs @ wkv
    k, v = (kv[..., :C].copy(), kv[..., C:].copy())
    scale = C ** (-0.5)
    p = _softmax(jnp.einsum('bqc,bkc->bqk', q, k) * scale, axis=-1)
    o = jnp.einsum('bqk,bkc->bqc', p, v) @ wo
    return o.reshape(B, H, W, C)
```

```python
import functools
import math
import numpy as np
import jax
import jax.numpy as jnp
from jax import lax
import jax.experimental.pallas as pl
import jax.experimental.pallas.tpu as pltpu

WIN = 8
F32 = jnp.float32
BF16 = jnp.bfloat16


def _nt(a, b):
    return lax.dot_general(a, b, (((1,), (1,)), ((), ())), preferred_element_type=F32)


def _nn(a, b):
    return lax.dot_general(a, b, (((1,), (0,)), ((), ())), preferred_element_type=F32)


def make(R=8, QB=512, KC=256, flags=None, NCH=6, summ='pair', D=0, lag=1, xlag=True):
    def fn(x, wq, wkv, wo):
        B, H, W, C = x.shape
        nh, nw = H // WIN, W // WIN
        NK = nh * nw
        n2 = H // R
        scale = (C ** -0.5) * math.log2(math.e)
        nt = W // 128
        per = QB // 128
        tiles = [(r, t) for r in range(R) for t in range(nt)]
        NB = len(tiles) // per
        HC = H // NCH
        NC = NK // KC

        def kernel(x_hbm, wq_ref, wkv_ref, wo_ref, o_ref, x_ref, xs_ref, k_ref, vt_ref, s_ref, m_ref, sems):
            i = pl.program_id(0)

            def load_x(row0, tl):
                return jnp.concatenate([x_ref[row0 + r, :, t * 128:(t + 1) * 128] for r, t in tl], axis=1)

            def stage_a(xt, slot, c, m):
                kc = pltpu.bitcast(k_ref[c * KC // 2:(c + 1) * KC // 2, :], BF16)
                s = _nn(kc[:, :C], xt)
                s_ref[slot, c * KC:(c + 1) * KC, :] = s
                for j in range(KC // 8):
                    sj = s[j * 8:(j + 1) * 8]
                    m = sj if m is None else jnp.maximum(m, sj)
                return m

            def stage_b(slot, c, m, l, acc):
                vt = pltpu.bitcast(vt_ref[:, c * KC:(c + 1) * KC], BF16)
                p = jnp.exp2(s_ref[slot, c * KC:(c + 1) * KC, :].reshape(KC // 8, 8, QB) - m)
                if summ == 'coarse':
                    lc = jnp.sum(p, axis=0)
                    l = lc if l is None else l + lc
                elif summ == 'chain':
                    for j in range(KC // 8):
                        l = p[j] if l is None else l + p[j]
                elif summ == 'pair':
                    for j in range(KC // 16):
                        t = p[2 * j] + p[2 * j + 1]
                        l = t if l is None else l + t
                pb = p.reshape(KC, QB).astype(BF16)
                o = _nn(vt, pb)
                return l, (o if acc is None else acc + o)

            @pl.when(i == 0)
            def _prologue():
                def cp(j):
                    return pltpu.make_async_copy(x_hbm.at[pl.ds(j * HC, HC)], x_ref.at[pl.ds(j * HC, HC)], sems.at[j])
                for j in range(NCH):
                    cp(j).start()
                r = lax.broadcasted_iota(jnp.int32, (nw, W), 0)
                c = lax.broadcasted_iota(jnp.int32, (nw, W), 1)
                pm = jnp.where((c >= r * WIN) & (c < r * WIN + WIN), 1.0, 0.0).astype(BF16)
                for j in range(NCH):
                    cp(j).wait()

                    def body(g, _):
                        acc = x_ref[g * WIN].astype(F32)
                        for t in range(1, WIN):
                            acc = acc + x_ref[g * WIN + t].astype(F32)
                        hi = acc.astype(BF16)
                        r1 = acc - hi.astype(F32)
                        mid = r1.astype(BF16)
                        xs = (_nt(pm, hi) + _nt(pm, mid)) * (1.0 / (WIN * WIN))
                        row = pl.multiple_of(g * nw, 16)
                        xs_ref[pl.ds(row, nw), :] = xs.astype(BF16)
                    lax.fori_loop(j * HC // WIN, (j + 1) * HC // WIN, body, None)
                xs = xs_ref[...]
                k = _nn(xs, wkv_ref[:, :C]).astype(BF16)
                v = _nn(xs, wkv_ref[:, C:]).astype(BF16)
                kk = (_nt(k, wq_ref[...]) * scale).astype(BF16)
                kk = jnp.concatenate([kk, jnp.zeros((NK, 128 - C), BF16)], axis=1)
                k_ref[...] = pltpu.bitcast(kk, jnp.uint32)
                vt_ref[...] = pltpu.bitcast(_nt(wo_ref[...].astype(F32).T.astype(BF16), v).astype(BF16), jnp.uint32)
                for b in range(NB):
                    xt = load_x(0, tiles[b * per:(b + 1) * per])
                    m = None
                    for c in range(NC):
                        m = stage_a(xt, b, c, m)
                    m_ref[b] = m

            nrow0 = jnp.minimum(i + 1, n2 - 1) * R
            lh = []
            mx = {}
            xc = {}
            m0s = [jnp.broadcast_to(jnp.max(m_ref[b], axis=0, keepdims=True), (8, QB)) for b in range(NB)]
            l = acc = None
            for t in range(NB * NC + D):
                if t < NB * NC:
                    b, c = divmod(t, NC)
                    if c == 0:
                        l = acc = None
                        if not xlag:
                            lh = []
                    m = m0s[b]
                    if lag and len(lh) >= lag:
                        m = jnp.where(lh[-lag] < 0, lh[-lag], m)
                    l, acc = stage_b(b, c, m, l, acc)
                    lh.append(l)
                    if c == NC - 1:
                        ls = jnp.sum(l, axis=0, keepdims=True)
                        o = (acc * (1.0 / ls)).astype(o_ref.dtype)
                        for j, (r, tt) in enumerate(tiles[b * per:(b + 1) * per]):
                            o_ref[r, :, tt * 128:(tt + 1) * 128] = o[:, j * 128:(j + 1) * 128]
                if t >= D:
                    ba, ca = divmod(t - D, NC)
                    if ba not in xc:
                        xc[ba] = load_x(nrow0, tiles[ba * per:(ba + 1) * per])
                    mx[ba] = stage_a(xc[ba], ba, ca, mx.get(ba))
                    if ca == NC - 1:
                        m_ref[ba] = mx[ba]

        xt = x.reshape(H, W, C).transpose(0, 2, 1)
        out = pl.pallas_call(
            kernel,
            grid=(n2,),
            in_specs=[
                pl.BlockSpec(memory_space=pl.ANY),
                pl.BlockSpec((C, C), lambda i: (0, 0)),
                pl.BlockSpec((C, 2 * C), lambda i: (0, 0)),
                pl.BlockSpec((C, C), lambda i: (0, 0)),
            ],
            out_specs=pl.BlockSpec((R, C, W), lambda i: (i, 0, 0)),
            out_shape=jax.ShapeDtypeStruct((H, C, W), x.dtype),
            scratch_shapes=[
                pltpu.VMEM((H, C, W), BF16),
                pltpu.VMEM((NK, C), BF16),
                pltpu.VMEM((NK // 2, 128), jnp.uint32),
                pltpu.VMEM((C // 2, NK), jnp.uint32),
                pltpu.VMEM((NB, NK, QB), F32),
                pltpu.VMEM((NB, 8, QB), F32),
                pltpu.SemaphoreType.DMA((NCH,)),
            ],
            compiler_params=pltpu.CompilerParams(
                dimension_semantics=("arbitrary",), vmem_limit_bytes=110 * 2**20, flags=flags),
            name="twins",
        )(xt, wq, wkv, wo)
        return out.transpose(0, 2, 1).reshape(B, H, W, C)
    return fn


@jax.jit
def pallas_standalone__window_attn_twins__vision_kernel(x, wq, wkv, wo):
    return make()(x, wq, wkv, wo)
```

```python
import math

import jax
import jax.numpy as jnp
from jax import lax
import jax.experimental.pallas as pl
import jax.experimental.pallas.tpu as pltpu

F32, BF16, U32 = jnp.float32, jnp.bfloat16, jnp.uint32

WIN = 8
ROWS = 8
EARLY = 2
GROUP = 4
QG = GROUP * 128
T = (-1.1, -0.625, -0.2, 0.2, 0.625, 1.1)
N = len(T)
FACTORS = sorted(
    [("H", i, j) for i in range(N) for j in range(N) if i != j]
    + [("G", i, j) for i in range(N) for j in range(i + 1, N)]
    + [("D", i) for i in range(N)] + [("E", i) for i in range(N)],
    key=lambda f: (max(f[1:]), min(f[1:]), f))


def _nt(a, b):
    return lax.dot_general(a, b, (((1,), (1,)), ((), ())), preferred_element_type=F32)


def _nn(a, b):
    return lax.dot_general(a, b, (((1,), (0,)), ((), ())), preferred_element_type=F32)


def _bf16(words):
    return pltpu.bitcast(words, BF16)


def _tile(q):
    return slice(q * 128, (q + 1) * 128)


def _span(j, size, align):
    return pl.ds(j * size if isinstance(j, int) else pl.multiple_of(j * size, align), size)


def _group_of(block, j):
    return (block * N + j) // GROUP


def _plan(groups, nk, kc, product_cycles, lead, tail):
    todo = []
    if product_cycles:
        todo = sorted((_group_of(n, 0 if f[0] == "D" else f[-1]), n, r)
                      for n in range(groups * GROUP // N) for r, f in enumerate(FACTORS))
    first = [sum(z[0] < g for z in todo) for g in range(groups + 1)]
    start = first[1] * product_cycles
    period = (groups * nk + len(todo) * product_cycles - start - tail) / groups
    units, marks, pace = [], [], []
    ia = ic = now = 0
    while ia < groups * nk:
        pick_c = False
        if ic < len(todo):
            g = todo[ic][0]
            due = start + (g - 1.1 + (ic - first[g]) / (first[g + 1] - first[g])) * period
            pick_c = ic % 10 > 0 or g <= ia // nk or due <= now
        while len(pace) * 16 < groups * nk and ic >= first[len(pace) * 16 // nk + 1]:
            due = start + len(pace) * 16 / nk * period
            if due > now and (pick_c or len(pace) * 16 >= ia + kc):
                break
            ready = [m for t, m in marks if t <= due - lead]
            pace.append(ready[-1] if ready else None)
        if pick_c:
            now += product_cycles
            marks.append((now, (len(units), 40)))
            units.append(("C",) + todo[ic][1:])
            ic += 1
        else:
            marks += [(now + r + 8, (len(units), r)) for r in range(0, kc, 16)]
            units.append(("A", ia // nk, ia % nk // kc))
            now += kc
            ia += kc
    assert ic == len(todo) and len(pace) * 16 == groups * nk
    return units, pace


@jax.jit
def pallas_standalone__window_attn_twins__vision_kernel(
    x: jax.Array,
    wq: jax.Array,
    wkv: jax.Array,
    wo: jax.Array,
):
    B, H, W, C = x.shape
    assert (B, H, W, C) == (1, 384, 384, 96)
    nw = W // WIN
    NK = (H // WIN) * nw
    KC = 8 * nw
    NC = NK // KC
    WT = W // 128
    NG = ROWS * WT // GROUP
    NB = ROWS * WT // N
    EG = EARLY * NG
    LAST = H // ROWS - 2
    scale = C ** -0.5 * math.log2(math.e)
    main_plan = _plan(NG, NK, KC, (C // 2) * (NK // N // 128) // 4, 190, 400)
    fill_plan = _plan(NG // 2, NK, KC, 0, 160, 300)

    def kernel(x_hbm, wq_hbm, wkv_hbm, wo_hbm, o_hbm,
               x_ref, wq_ref, wkv_ref, wo_ref, wk_ref, wvt_ref, xs_ref, xg_ref, k_ref, v_ref, vf_ref,
               s_ref, max_ref, p_ref, l_ref, es_ref, eo_ref, em_ref, el_ref, o_ref, xsem, wsem, osem):

        def x_copy(j):
            rows = pl.ds(j * (H // NC), H // NC)
            return pltpu.make_async_copy(x_hbm.at[rows], x_ref.at[rows], xsem.at[j])

        def o_copy(step):
            return pltpu.make_async_copy(
                o_ref.at[step % 4], o_hbm.at[pl.ds(step * ROWS, ROWS)], osem.at[step % 4])

        def o_last_copies(part):
            row, n = part * (ROWS // 4), ROWS // 4
            return [pltpu.make_async_copy(
                o_ref.at[step % 4, pl.ds(row, n)], o_hbm.at[pl.ds(step * ROWS + row, n)],
                osem.at[4 + 2 * part + step % 2]) for step in (LAST, LAST + 1)]

        def load_x(row0, g):
            tiles = range(g * GROUP, (g + 1) * GROUP)
            return jnp.concatenate([x_ref[row0 + q // WT, :, _tile(q % WT)] for q in tiles], axis=1)

        def store_o(slot, row0, q, o):
            o_ref[slot, row0 + q // WT, :, _tile(q % WT)] = o.astype(o_ref.dtype)

        def after(i, dep, val):
            never = (lax.broadcasted_iota(jnp.int32, (8, 128), 0) + i < 0)[None]
            dep = lax.bitcast_convert_type(dep, val.dtype).reshape(-1, 8, 128)
            cols = [jnp.where(never, dep, val[None, :, _tile(q)]) for q in range(val.shape[1] // 128)]
            return jnp.concatenate(cols, axis=2).reshape(-1, val.shape[1])

        def sublane_max(s):
            return jnp.max(s.reshape(KC // 8, 8, QG), axis=0)

        def row_max(g):
            return jnp.max(jnp.max(max_ref[g], axis=0), axis=0, keepdims=True)

        def inv_sum(l):
            return 1.0 / jnp.sum(l, axis=0, keepdims=True)

        def window_means(pool, r):
            acc = x_ref[r * WIN].astype(F32)
            for i in range(1, WIN):
                acc = acc + x_ref[r * WIN + i].astype(F32)
            acc = acc.astype(BF16)
            sums = [_nt(pool, acc[:, _tile(q)]) for q in range(WT)]
            return jnp.concatenate(sums, axis=0) * (1.0 / (WIN * WIN))

        def project(j):
            xf = xs_ref[...]
            xs = xf.astype(BF16)
            k_ref[_span(j, KC // 2, 8), :] = pltpu.bitcast(_nn(xs, wk_ref[...]).astype(BF16), U32)
            v_ref[j] = pltpu.bitcast(_nt(wvt_ref[...], xs).astype(BF16), U32)
            n = KC // N
            xf = xf.reshape(n // 16, N, 16, C)
            for i in range(N):
                xg_ref[i, _span(j, n, 16), :] = xf[:, i].reshape(n, C).astype(BF16)

        def value_factors(values):
            v = _nt(wvt_ref[...], xg_ref[len(values)])
            values.append((v[:C // 2], v[C // 2:] + T[len(values)] * v[:C // 2]))
            top, mix = zip(*values)
            for r, f in enumerate(FACTORS):
                i, j = min(f[1:]), max(f[1:])
                if j != len(values) - 1:
                    continue
                if i == j:
                    val = top[i] if f[0] == "D" else mix[i]
                else:
                    val = ((mix[j] - mix[i]) * (1.0 / (T[j] - T[i]))).astype(BF16).astype(F32)
                if f[0] == "H":
                    val = val - top[i] if f[1] == i and (i + j) % 2 else top[f[1]] - val
                vf_ref[r] = pltpu.bitcast(val.astype(BF16), U32)

        def keys(j):
            return _bf16(k_ref[_span(j, KC // 2, 8), :])[:, :C]

        def plain_pv(s, m, l, j):
            p = jnp.exp2(s.reshape(KC // 16, 2, 8, QG) - m)
            pairs = p[:, 0] + p[:, 1]
            for u in range(KC // 16):
                l = pairs[u] if l is None else l + pairs[u]
            return l, _nn(_bf16(v_ref[j]), p.reshape(KC, QG).astype(BF16))

        def online(e, j, chunk_max):
            m_old = em_ref[e]
            m = jnp.maximum(m_old, jnp.max(chunk_max, axis=0, keepdims=True))
            alpha = jnp.exp2(m_old - m)
            l, o = plain_pv(es_ref[e], m, el_ref[e] * alpha, j)
            return m, l, (eo_ref[e].reshape(C // 8, 8, QG) * alpha).reshape(C, QG) + o

        def finish_chunk(j, valid, side_work):
            k = keys(j)
            for g in range(NG):
                side_work(g)
                s = _nn(k, load_x(EARLY * ROWS, g))
                s_ref[g, _span(j, KC, 8), :] = s
                max_ref[g, j] = sublane_max(s)
                if g == 0:
                    m, l, o = online(EG - 1, j, em_ref[EG])
                    em_ref[EG - 1] = jnp.where(valid, m, -jnp.inf)
                    el_ref[EG - 1] = jnp.where(valid, l, 0.0)
                    eo_ref[EG - 1] = o

        def stream_chunk(j, pool):
            x_copy(j).wait()

            def build(g):
                for r, at in enumerate((1, 2, 3, 3, 4, 4, 5, 5)):
                    if at == g:
                        xs_ref[r * nw:(r + 1) * nw, :] = window_means(pool, 8 * j + r)
                if g == NG - 1:
                    project(j)
            finish_chunk(jnp.maximum(j - 1, 0), j > 0, build)
            k = keys(j)
            for e in range(EG):
                s = _nn(k, load_x(0, e))
                es_ref[e] = s
                if e:
                    em_ref[e - 1], el_ref[e - 1], eo_ref[e - 1] = online(e - 1, j, chunk_max)
                chunk_max = sublane_max(s)
            em_ref[EG] = chunk_max

        def exp_offset(g):
            m = row_max(g)
            part = jnp.sum(jnp.sum(jnp.exp2(max_ref[g] - m), axis=0), axis=0, keepdims=True)
            power = (lax.bitcast_convert_type(part, jnp.int32) >> 23) - 127
            return jnp.broadcast_to(m + power.astype(F32), (8, QG))

        def stage_b(n0, g, s, m):
            runs = NK // (16 * N)
            p = jnp.exp2(s.reshape(runs, N, 2, 8, QG) - m.reshape(runs, N, 1, 8, QG))
            p = [p[:, i].reshape(NK // N, QG) for i in range(N)]

            def put(n, f, val):
                p_ref[n0 + n, FACTORS.index(f)] = val.astype(BF16)

            def get(n, f):
                return p_ref[n0 + n, FACTORS.index(f)].astype(F32)

            col = p[0]
            for i in range(N):
                col = col + p[i] if i else col
                terms = {}
                for w in range(GROUP):
                    n, j = divmod(g * GROUP + w, N)
                    cur = p[i][:, _tile(w)]
                    terms.setdefault(n, []).append((i != j and (i + j) % 2 == 0, cur))
                    if i != j:
                        put(n, ("H", i, j), cur)
                    if i != j and (_group_of(n, i), j) < (g, i):
                        same = _group_of(n, i) == g
                        other = p[j][:, _tile(w + i - j)] if same else get(n, ("H", j, i))
                        hi, lo = (cur, other) if i > j else (other, cur)
                        put(n, ("G", min(i, j), max(i, j)), hi - lo if (i + j) % 2 else hi + lo)
                for n, row in terms.items():
                    if _group_of(n, 0) < g:
                        row = [(False, get(n, ("D", i)))] + row
                    row = sorted(row, key=lambda z: z[0])
                    assert not row[0][0]
                    val = row[0][1]
                    for minus, z in row[1:]:
                        val = val - z if minus else val + z
                    put(n, ("D", i), val)
            for w in range(GROUP):
                n, j = divmod(g * GROUP + w, N)
                put(n, ("E", j), col[:, _tile(w)])
            col = col.reshape(runs, 2, 8, QG)
            col = col[:, 0] + col[:, 1]
            l = col[0]
            for u in range(1, runs):
                l = l + col[u]
            return l

        def stage_c(slot, row0, n0, n, r, done, inv, pin=None):
            vf = vf_ref[r]
            if pin is not None:
                head = jnp.concatenate([pin(vf[:8, :128]), vf[:8, 128:]], axis=1)
                vf = jnp.concatenate([head, vf[8:]], axis=0)
            f = FACTORS[r]
            res = _nn(_bf16(vf), p_ref[n0 + n, r])
            done[(n,) + f] = res
            i, j = min(f[1:]), max(f[1:])
            if all(z in done for z in ((n, "G", i, j), (n, "H", i, j), (n, "H", j, i))):
                done[n, "Z", i, j] = done[n, "H", j, i] + done[n, "H", i, j] + done[n, "G", i, j]
            for q in sorted(f[1:]):
                others = [z for z in range(N) if z != q]
                if ((n, "D", q) in done and (n, "E", q) in done
                        and all((n, "Z", min(q, z), max(q, z)) in done for z in others)):
                    top, bot = done[n, "D", q], done[n, "E", q]
                    for z in others:
                        minus = z < q and (z + q) % 2 == 1
                        zz = done[n, "Z", min(q, z), max(q, z)]
                        top = top - zz if minus else top + zz
                        bot = bot + (T[z] - T[q] if minus else T[q] - T[z]) * done[n, "H", z, q]
                    g, w = divmod(n * N + q, GROUP)
                    o = jnp.concatenate([top, bot - T[q] * top], axis=0) * inv[g][:, _tile(w)]
                    store_o(slot, row0, n * N + q, o)
            return res

        def run(plan, groups, row0, slot, g0=0, n0=0):
            units, pace = plan
            offs = [exp_offset(g0 + g) for g in range(groups)]
            inv = None if slot is None else [inv_sum(l_ref[g]) for g in range(groups)]
            done, out = {}, []
            for kind, a, b in units:
                if kind == "C":
                    g, w = divmod(len(out) - 4, GROUP)
                    pin = None
                    if 0 <= g < groups:
                        pin = lambda v: after(
                            row0, jnp.broadcast_to(inv[g][:, _tile(w)], (8, 128)),
                            after(row0, offs[g][:, _tile(w)], v))
                    out.append(stage_c(slot, 0, n0, a, b, done, inv, pin))
                    continue
                if b == 0:
                    xt, s_old = load_x(row0, a), s_ref[g0 + a]
                s = _nn(keys(b), xt)
                s_ref[g0 + a, b * KC:(b + 1) * KC, :] = s
                max_ref[g0 + a, b] = sublane_max(s)
                out.append(s)
                if b == NC - 1:
                    marks = pace[a * NK // 16:(a + 1) * NK // 16]
                    free = [offs[a] for z in marks if z is None]
                    deps = jnp.concatenate([out[u][r:r + 8, :128] for u, r in marks[len(free):]], axis=0)
                    off = jnp.concatenate(free + [after(row0, deps, offs[a])], axis=0)
                    l_ref[g0 + a] = stage_b(n0, a, s_old, off)

        def fill(half, _):
            row0 = (EARLY + 1) * ROWS + half * (ROWS // 2)
            run(fill_plan, NG // 2, row0, None, half * (NG // 2), half * (NB // 2))

        def step(i, _):
            o_copy(i - EARLY).wait()
            run(main_plan, NG, (i + 2) * ROWS, i % 4)
            o_copy(i).start()

        def drain(half, _):
            groups, g0, n0, row0 = NG // 2, half * (NG // 2), half * (NB // 2), half * (ROWS // 2)
            inv = [inv_sum(l_ref[g0 + g]) for g in range(groups)]
            total = NB // 2 * len(FACTORS)
            done, ic, prev = {}, 0, None
            for g in range(groups):
                m = jnp.broadcast_to(row_max(g0 + g), (8, QG))
                l = o = None
                for j in range(NC):
                    while ic < total and (ic % 4 or ic * groups * NC < (g * NC + j + 1) * total):
                        stage_c(LAST % 4, row0, n0, *divmod(ic, len(FACTORS)), done, inv)
                        ic += 1
                    mj = m if prev is None else after(half, prev[:, -128:], m)
                    l, part = plain_pv(s_ref[g0 + g, j * KC:(j + 1) * KC, :], mj, l, j)
                    o, prev = part if o is None else o + part, l
                o = o * inv_sum(l)
                for w in range(GROUP):
                    store_o((LAST + 1) % 4, row0, g * GROUP + w, o[:, _tile(w)])
                if g:
                    for cp in o_last_copies(2 * half + g - 1):
                        cp.start()

        weights = [pltpu.make_async_copy(src, dst, wsem.at[i]) for i, (src, dst) in
                   enumerate([(wq_hbm, wq_ref), (wkv_hbm, wkv_ref), (wo_hbm, wo_ref)])]
        for cp in weights:
            cp.start()
        lax.fori_loop(0, NC, lambda j, _: x_copy(j).start(), None)

        win = lax.broadcasted_iota(jnp.int32, (128 // WIN, 128), 0) * WIN
        pos = lax.broadcasted_iota(jnp.int32, (128 // WIN, 128), 1)
        pool = jnp.where((pos >= win) & (pos < win + WIN), 1.0, 0.0).astype(BF16)
        em_ref[:EG] = jnp.full((EG, 8, QG), -jnp.inf, F32)
        em_ref[EG] = jnp.zeros((8, QG), F32)
        el_ref[...] = jnp.zeros(el_ref.shape, F32)
        eo_ref[...] = jnp.zeros(eo_ref.shape, F32)
        es_ref[EG - 1] = jnp.zeros((KC, QG), F32)
        k_ref[:KC // 2] = jnp.zeros((KC // 2, 128), U32)
        v_ref[0] = jnp.zeros((C // 2, KC), U32)
        for cp in weights:
            cp.wait()
        wk = (_nt(wkv_ref[:, :C], wq_ref[...]) * scale).astype(BF16)
        wk_ref[...] = jnp.concatenate([wk, jnp.zeros((C, 128 - C), BF16)], axis=1)
        wvt_ref[...] = _nn(wkv_ref[:, C:], wo_ref[...]).T.astype(BF16)

        lax.fori_loop(0, NC, lambda j, _: stream_chunk(j, pool), None)
        values = []
        finish_chunk(NC - 1, True, lambda g: value_factors(values))
        assert len(values) == N
        for e in range(EG):
            o = eo_ref[e] * inv_sum(el_ref[e])
            for w in range(GROUP):
                store_o(e // NG, 0, e % NG * GROUP + w, o[:, _tile(w)])
        for i in range(EARLY):
            o_copy(i).start()

        lax.fori_loop(0, 2, fill, None)
        lax.fori_loop(EARLY, LAST, step, None)
        lax.fori_loop(0, 2, drain, None)
        for i in range(LAST - EARLY, LAST):
            o_copy(i).wait()
        for part in range(4):
            for cp in o_last_copies(part):
                cp.wait()

    out = pl.pallas_call(
        kernel,
        in_specs=[pl.BlockSpec(memory_space=pl.ANY)] * 4,
        out_specs=pl.BlockSpec(memory_space=pl.ANY),
        out_shape=jax.ShapeDtypeStruct((H, C, W), x.dtype),
        scratch_shapes=[
            pltpu.VMEM((H, C, W), BF16),
            pltpu.VMEM((C, C), BF16),
            pltpu.VMEM((C, 2 * C), BF16),
            pltpu.VMEM((C, C), BF16),
            pltpu.VMEM((C, 128), BF16),
            pltpu.VMEM((C, C), BF16),
            pltpu.VMEM((KC, C), F32),
            pltpu.VMEM((N, NK // N, C), BF16),
            pltpu.VMEM((NK // 2, 128), U32),
            pltpu.VMEM((NC, C // 2, KC), U32),
            pltpu.VMEM((len(FACTORS), C // 4, NK // N), U32),
            pltpu.VMEM((NG, NK, QG), F32),
            pltpu.VMEM((NG, NC, 8, QG), F32),
            pltpu.VMEM((NB, len(FACTORS), NK // N, 128), BF16),
            pltpu.VMEM((NG, 8, QG), F32),
            pltpu.VMEM((EG, KC, QG), F32),
            pltpu.VMEM((EG, C, QG), F32),
            pltpu.VMEM((EG + 1, 8, QG), F32),
            pltpu.VMEM((EG, 8, QG), F32),
            pltpu.VMEM((4, ROWS, C, W), BF16),
            pltpu.SemaphoreType.DMA((NC,)),
            pltpu.SemaphoreType.DMA((3,)),
            pltpu.SemaphoreType.DMA((12,)),
        ],
        compiler_params=pltpu.CompilerParams(vmem_limit_bytes=110 * 2**20),
    )(x.reshape(H, W, C).transpose(0, 2, 1), wq, wkv, wo)
    return out.transpose(0, 2, 1).reshape(B, H, W, C)
```

```python
import math

import jax
import jax.numpy as jnp
from jax import lax
import jax.experimental.pallas as pl
import jax.experimental.pallas.tpu as pltpu

F32, BF16, U32 = jnp.float32, jnp.bfloat16, jnp.uint32

WIN = 8
ROWS = 8
EARLY = 2
GROUP = 4
QG = GROUP * 128
T = (-1.1, -0.625, -0.2, 0.2, 0.625, 1.1)
N = len(T)
FACTORS = sorted(
    [("H", i, j) for i in range(N) for j in range(N) if i != j]
    + [("G", i, j) for i in range(N) for j in range(i + 1, N)]
    + [("D", i) for i in range(N)] + [("E", i) for i in range(N)],
    key=lambda f: (max(f[1:]), min(f[1:]), f))


def _nt(a, b):
    return lax.dot_general(a, b, (((1,), (1,)), ((), ())), preferred_element_type=F32)


def _nn(a, b):
    return lax.dot_general(a, b, (((1,), (0,)), ((), ())), preferred_element_type=F32)


def _bf16(words):
    return pltpu.bitcast(words, BF16)


def _tile(q):
    return slice(q * 128, (q + 1) * 128)


def _span(j, size, align):
    return pl.ds(j * size if isinstance(j, int) else pl.multiple_of(j * size, align), size)


def _group_of(block, j):
    return (block * N + j) // GROUP


def _writer(block, r):
    return _group_of(block, 0 if FACTORS[r][0] == "D" else FACTORS[r][-1])


SLOTS = sorted(((n, r) for n in range(2) for r in range(len(FACTORS))),
               key=lambda z: (_writer(*z), FACTORS[z[1]][0] == "D", z))


def _plan(groups, nk, kc, product_cycles, lead, tail):
    todo = []
    if product_cycles:
        todo = sorted((_writer(n, r), n, r)
                      for n in range(groups * GROUP // N) for r in range(len(FACTORS)))
    first = [sum(z[0] < g for z in todo) for g in range(groups + 1)]
    start = first[1] * product_cycles
    period = (groups * nk + len(todo) * product_cycles - start - tail) / groups
    units, marks, pace = [], [], []
    ia = ic = now = 0
    while ia < groups * nk:
        pick_c = False
        if ic < len(todo):
            g = todo[ic][0]
            due = start + (g - 1.06 + (ic - first[g]) / (first[g + 1] - first[g])) * period
            pick_c = ic % 12 > 0 or g <= ia // nk or due <= now
        while len(pace) * 16 < groups * nk and ic >= first[len(pace) * 16 // nk + 1]:
            due = start + len(pace) * 16 / nk * period
            if due > now and (pick_c or len(pace) * 16 >= ia + kc):
                break
            ready = [m for t, m in marks if t <= due - lead]
            pace.append(ready[-1] if ready else None)
        if pick_c:
            now += product_cycles
            marks.append((now, (len(units), 40)))
            units.append(("C",) + todo[ic][1:])
            ic += 1
        else:
            marks += [(now + r + 8, (len(units), r)) for r in range(0, kc, 16)]
            units.append(("A", ia // nk, ia % nk // kc))
            now += kc
            ia += kc
    assert ic == len(todo) and len(pace) * 16 == groups * nk
    return units, pace


@jax.jit
def pallas_standalone__window_attn_twins__vision_kernel(
    x: jax.Array,
    wq: jax.Array,
    wkv: jax.Array,
    wo: jax.Array,
):
    B, H, W, C = x.shape
    assert (B, H, W, C) == (1, 384, 384, 96)
    nw = W // WIN
    NK = (H // WIN) * nw
    KC = 8 * nw
    NC = NK // KC
    WT = W // 128
    NG = ROWS * WT // GROUP
    EG = EARLY * NG
    LAST = H // ROWS - 2
    scale = C ** -0.5 * math.log2(math.e)
    main_plan = _plan(NG, NK, KC, (C // 2) * (NK // N // 128) // 4, 270, 600)
    fill_plan = _plan(NG // 2, NK, KC, 0, 350, 300)

    def kernel(x_hbm, wq_hbm, wkv_hbm, wo_hbm, o_hbm,
               x_ref, wq_ref, wkv_ref, wo_ref, wk_ref, wvt_ref, xs_ref, xg_ref, k_ref, v_ref, vf_ref,
               s_ref, max_ref, p_ref, l_ref, es_ref, eo_ref, em_ref, el_ref, o_ref, xsem, wsem, osem):

        def x_copy(j):
            rows = pl.ds(j * (H // NC), H // NC)
            return pltpu.make_async_copy(x_hbm.at[rows], x_ref.at[rows], xsem.at[j])

        def o_copy(step):
            return pltpu.make_async_copy(
                o_ref.at[step % 4], o_hbm.at[pl.ds(step * ROWS, ROWS)], osem.at[step % 4])

        def o_last_copies(part):
            row, n = part * (ROWS // 4), ROWS // 4
            return [pltpu.make_async_copy(
                o_ref.at[step % 4, pl.ds(row, n)], o_hbm.at[pl.ds(step * ROWS + row, n)],
                osem.at[4 + 2 * part + step % 2]) for step in (LAST, LAST + 1)]

        def load_x(row0, g):
            tiles = range(g * GROUP, (g + 1) * GROUP)
            return jnp.concatenate([x_ref[row0 + q // WT, :, _tile(q % WT)] for q in tiles], axis=1)

        def store_o(slot, row0, q, o):
            o_ref[slot, row0 + q // WT, :, _tile(q % WT)] = o.astype(o_ref.dtype)

        def after(i, dep, val):
            never = (lax.broadcasted_iota(jnp.int32, (8, 128), 0) + i < 0)[None]
            dep = lax.bitcast_convert_type(dep, val.dtype).reshape(-1, 8, 128)
            cols = [jnp.where(never, dep, val[None, :, _tile(q)]) for q in range(val.shape[1] // 128)]
            return jnp.concatenate(cols, axis=2).reshape(-1, val.shape[1])

        def sublane_max(s):
            return jnp.max(s.reshape(KC // 8, 8, QG), axis=0)

        def row_max(g):
            return jnp.max(jnp.max(max_ref[g], axis=0), axis=0, keepdims=True)

        def inv_sum(l):
            return 1.0 / jnp.sum(l, axis=0, keepdims=True)

        def window_means(pool, r):
            acc = x_ref[r * WIN].astype(F32)
            for i in range(1, WIN):
                acc = acc + x_ref[r * WIN + i].astype(F32)
            acc = acc.astype(BF16)
            sums = [_nt(pool, acc[:, _tile(q)]) for q in range(WT)]
            return jnp.concatenate(sums, axis=0) * (1.0 / (WIN * WIN))

        def project(j):
            xf = xs_ref[...]
            xs = xf.astype(BF16)
            k_ref[_span(j, KC // 2, 8), :] = pltpu.bitcast(_nn(xs, wk_ref[...]).astype(BF16), U32)
            v_ref[j] = pltpu.bitcast(_nt(wvt_ref[...], xs).astype(BF16), U32)
            n = KC // N
            xf = xf.reshape(n // 16, N, 16, C)
            for i in range(N):
                xg_ref[i, _span(j, n, 16), :] = xf[:, i].reshape(n, C).astype(BF16)

        def value_factors(values):
            v = _nt(wvt_ref[...], xg_ref[len(values)])
            values.append((v[:C // 2], v[C // 2:] + T[len(values)] * v[:C // 2]))
            top, mix = zip(*values)
            for r, f in enumerate(FACTORS):
                i, j = min(f[1:]), max(f[1:])
                if j != len(values) - 1:
                    continue
                if i == j:
                    val = top[i] if f[0] == "D" else mix[i]
                else:
                    val = ((mix[j] - mix[i]) * (1.0 / (T[j] - T[i]))).astype(BF16).astype(F32)
                if f[0] == "H":
                    val = val - top[i] if f[1] == i and (i + j) % 2 else top[f[1]] - val
                vf_ref[r] = pltpu.bitcast(val.astype(BF16), U32)

        def keys(j):
            return _bf16(k_ref[_span(j, KC // 2, 8), :])[:, :C]

        def plain_pv(s, m, l, j):
            p = jnp.exp2(s.reshape(KC // 16, 2, 8, QG) - m)
            pairs = p[:, 0] + p[:, 1]
            for u in range(KC // 16):
                l = pairs[u] if l is None else l + pairs[u]
            return l, _nn(_bf16(v_ref[j]), p.reshape(KC, QG).astype(BF16))

        def online(e, j, chunk_max):
            m_old = em_ref[e]
            m = jnp.maximum(m_old, jnp.max(chunk_max, axis=0, keepdims=True))
            alpha = jnp.exp2(m_old - m)
            l, o = plain_pv(es_ref[e], m, el_ref[e] * alpha, j)
            return m, l, (eo_ref[e].reshape(C // 8, 8, QG) * alpha).reshape(C, QG) + o

        def finish_chunk(j, valid, side_work):
            k = keys(j)
            for g in range(NG):
                side_work(g)
                s = _nn(k, load_x(EARLY * ROWS, g))
                s_ref[g, _span(j, KC, 8), :] = s
                max_ref[g, j] = sublane_max(s)
                if g == 0:
                    m, l, o = online(EG - 1, j, em_ref[EG])
                    em_ref[EG - 1] = jnp.where(valid, m, -jnp.inf)
                    el_ref[EG - 1] = jnp.where(valid, l, 0.0)
                    eo_ref[EG - 1] = o

        def stream_chunk(j, pool):
            x_copy(j).wait()

            def build(g):
                for r, at in enumerate((1, 2, 3, 3, 4, 4, 5, 5)):
                    if at == g:
                        xs_ref[r * nw:(r + 1) * nw, :] = window_means(pool, 8 * j + r)
                if g == NG - 1:
                    project(j)
            finish_chunk(jnp.maximum(j - 1, 0), j > 0, build)
            k = keys(j)
            for e in range(EG):
                s = _nn(k, load_x(0, e))
                es_ref[e] = s
                if e:
                    em_ref[e - 1], el_ref[e - 1], eo_ref[e - 1] = online(e - 1, j, chunk_max)
                chunk_max = sublane_max(s)
            em_ref[EG] = chunk_max

        def exp_offset(g):
            m = row_max(g)
            part = jnp.sum(jnp.sum(jnp.exp2(max_ref[g] - m), axis=0), axis=0, keepdims=True)
            power = (lax.bitcast_convert_type(part, jnp.int32) >> 23) - 127
            return jnp.broadcast_to(m + power.astype(F32), (8, QG))

        def stage_b(half, g, s, m):
            runs = NK // (16 * N)
            p = jnp.exp2(s.reshape(runs, N, 2, 8, QG) - m.reshape(runs, N, 1, 8, QG))
            p = [p[:, i].reshape(NK // N, QG) for i in range(N)]

            made = {}

            def put(n, f, val):
                made[SLOTS.index((n, FACTORS.index(f)))] = val.astype(BF16)[None]

            def get(n, f):
                return p_ref[half, SLOTS.index((n, FACTORS.index(f)))].astype(F32)

            col = p[0]
            for i in range(N):
                col = col + p[i] if i else col
                terms = {}
                for w in range(GROUP):
                    n, j = divmod(g * GROUP + w, N)
                    cur = p[i][:, _tile(w)]
                    terms.setdefault(n, []).append((i != j and (i + j) % 2 == 0, cur))
                    if i != j:
                        put(n, ("H", i, j), cur)
                    if i != j and (_group_of(n, i), j) < (g, i):
                        same = _group_of(n, i) == g
                        other = p[j][:, _tile(w + i - j)] if same else get(n, ("H", j, i))
                        hi, lo = (cur, other) if i > j else (other, cur)
                        put(n, ("G", min(i, j), max(i, j)), hi - lo if (i + j) % 2 else hi + lo)
                for n, row in terms.items():
                    if _group_of(n, 0) < g:
                        row = [(False, get(n, ("D", i)))] + row
                    row = sorted(row, key=lambda z: z[0])
                    assert not row[0][0]
                    val = row[0][1]
                    for minus, z in row[1:]:
                        val = val - z if minus else val + z
                    put(n, ("D", i), val)
            for w in range(GROUP):
                n, j = divmod(g * GROUP + w, N)
                put(n, ("E", j), col[:, _tile(w)])
            lo, hi = min(made), max(made) + 1
            p_ref[half, lo:hi] = jnp.concatenate([made[z] for z in range(lo, hi)], axis=0)
            col = col.reshape(runs, 2, 8, QG)
            col = col[:, 0] + col[:, 1]
            l = col[0]
            for u in range(1, runs):
                l = l + col[u]
            return l

        def stage_c(slot, row0, n, r, vf, pf, done, inv, pin=None):
            vf = vf[r]
            if pin is not None:
                head = jnp.concatenate([pin(vf[:8, :128]), vf[:8, 128:]], axis=1)
                vf = jnp.concatenate([head, vf[8:]], axis=0)
            f = FACTORS[r]
            res = _nn(_bf16(vf), pf[SLOTS.index((n % 2, r))])
            done[(n,) + f] = res
            i, j = min(f[1:]), max(f[1:])
            if all(z in done for z in ((n, "G", i, j), (n, "H", i, j), (n, "H", j, i))):
                done[n, "Z", i, j] = done[n, "H", j, i] + done[n, "H", i, j] + done[n, "G", i, j]
            for q in sorted(f[1:]):
                others = [z for z in range(N) if z != q]
                if ((n, "D", q) in done and (n, "E", q) in done
                        and all((n, "Z", min(q, z), max(q, z)) in done for z in others)):
                    top, bot = done[n, "D", q], done[n, "E", q]
                    for z in others:
                        minus = z < q and (z + q) % 2 == 1
                        zz = done[n, "Z", min(q, z), max(q, z)]
                        top = top - zz if minus else top + zz
                        bot = bot + (T[z] - T[q] if minus else T[q] - T[z]) * done[n, "H", z, q]
                    g, w = divmod(n * N + q, GROUP)
                    o = jnp.concatenate([top, bot - T[q] * top], axis=0) * inv[g][:, _tile(w)]
                    store_o(slot, row0, n * N + q, o)
            return res

        def run(plan, groups, row0, slot, half=0):
            units, pace = plan
            g0 = half * (NG // 2)
            offs = [exp_offset(g0 + g) for g in range(groups)]
            if slot is not None:
                inv = [inv_sum(l_ref[g]) for g in range(groups)]
                vf, pf = vf_ref[...], (p_ref[0], p_ref[1])
            done, out = {}, []
            for kind, a, b in units:
                if kind == "C":
                    g, w = divmod(len(out) - 4, GROUP)
                    pin = None
                    if 0 <= g < groups:
                        pin = lambda v: after(
                            row0, jnp.broadcast_to(inv[g][:, _tile(w)], (8, 128)),
                            after(row0, offs[g][:, _tile(w)], v))
                    out.append(stage_c(slot, 0, a, b, vf, pf[a // 2], done, inv, pin))
                    continue
                if b == 0:
                    xt, s_old = load_x(row0, a), s_ref[g0 + a]
                s = _nn(keys(b), xt)
                s_ref[g0 + a, b * KC:(b + 1) * KC, :] = s
                max_ref[g0 + a, b] = sublane_max(s)
                out.append(s)
                if b == NC - 1:
                    marks = pace[a * NK // 16:(a + 1) * NK // 16]
                    free = [offs[a] for z in marks if z is None]
                    deps = jnp.concatenate([out[u][r:r + 8, :128] for u, r in marks[len(free):]], axis=0)
                    off = jnp.concatenate(free + [after(row0, deps, offs[a])], axis=0)
                    l_ref[g0 + a] = stage_b(half + a // 3, a % 3, s_old, off)

        def fill(half, _):
            row0 = (EARLY + 1) * ROWS + half * (ROWS // 2)
            run(fill_plan, NG // 2, row0, None, half)

        def step(i, _):
            o_copy(i - EARLY).wait()
            run(main_plan, NG, (i + 2) * ROWS, i % 4)
            o_copy(i).start()

        def drain(half, _):
            groups, g0, row0 = NG // 2, half * (NG // 2), half * (ROWS // 2)
            inv = [inv_sum(l_ref[g0 + g]) for g in range(groups)]
            vf, pf, total = vf_ref[...], p_ref[half], len(SLOTS)
            done, ic, prev = {}, 0, None
            for g in range(groups):
                m = jnp.broadcast_to(row_max(g0 + g), (8, QG))
                l = o = None
                for j in range(NC):
                    while ic < total and (ic % 4 or ic * groups * NC < (g * NC + j + 1) * total):
                        stage_c(LAST % 4, row0, *divmod(ic, len(FACTORS)), vf, pf, done, inv)
                        ic += 1
                    mj = m if prev is None else after(half, prev[:, -128:], m)
                    l, part = plain_pv(s_ref[g0 + g, j * KC:(j + 1) * KC, :], mj, l, j)
                    o, prev = part if o is None else o + part, l
                o = o * inv_sum(l)
                for w in range(GROUP):
                    store_o((LAST + 1) % 4, row0, g * GROUP + w, o[:, _tile(w)])
                if g:
                    for cp in o_last_copies(2 * half + g - 1):
                        cp.start()

        weights = [pltpu.make_async_copy(src, dst, wsem.at[i]) for i, (src, dst) in
                   enumerate([(wq_hbm, wq_ref), (wkv_hbm, wkv_ref), (wo_hbm, wo_ref)])]
        for cp in weights:
            cp.start()
        lax.fori_loop(0, NC, lambda j, _: x_copy(j).start(), None)

        win = lax.broadcasted_iota(jnp.int32, (128 // WIN, 128), 0) * WIN
        pos = lax.broadcasted_iota(jnp.int32, (128 // WIN, 128), 1)
        pool = jnp.where((pos >= win) & (pos < win + WIN), 1.0, 0.0).astype(BF16)
        em_ref[:EG] = jnp.full((EG, 8, QG), -jnp.inf, F32)
        em_ref[EG] = jnp.zeros((8, QG), F32)
        el_ref[...] = jnp.zeros(el_ref.shape, F32)
        eo_ref[...] = jnp.zeros(eo_ref.shape, F32)
        es_ref[EG - 1] = jnp.zeros((KC, QG), F32)
        k_ref[:KC // 2] = jnp.zeros((KC // 2, 128), U32)
        v_ref[0] = jnp.zeros((C // 2, KC), U32)
        for cp in weights:
            cp.wait()
        wk = (_nt(wkv_ref[:, :C], wq_ref[...]) * scale).astype(BF16)
        wk_ref[...] = jnp.concatenate([wk, jnp.zeros((C, 128 - C), BF16)], axis=1)
        wvt_ref[...] = _nn(wkv_ref[:, C:], wo_ref[...]).T.astype(BF16)

        lax.fori_loop(0, NC, lambda j, _: stream_chunk(j, pool), None)
        values = []
        finish_chunk(NC - 1, True, lambda g: value_factors(values))
        assert len(values) == N
        for e in range(EG):
            o = eo_ref[e] * inv_sum(el_ref[e])
            for w in range(GROUP):
                store_o(e // NG, 0, e % NG * GROUP + w, o[:, _tile(w)])
        for i in range(EARLY):
            o_copy(i).start()

        lax.fori_loop(0, 2, fill, None)
        lax.fori_loop(EARLY, LAST, step, None)
        lax.fori_loop(0, 2, drain, None)
        for i in range(LAST - EARLY, LAST):
            o_copy(i).wait()
        for part in range(4):
            for cp in o_last_copies(part):
                cp.wait()

    out = pl.pallas_call(
        kernel,
        in_specs=[pl.BlockSpec(memory_space=pl.ANY)] * 4,
        out_specs=pl.BlockSpec(memory_space=pl.ANY),
        out_shape=jax.ShapeDtypeStruct((H, C, W), x.dtype),
        scratch_shapes=[
            pltpu.VMEM((H, C, W), BF16),
            pltpu.VMEM((C, C), BF16),
            pltpu.VMEM((C, 2 * C), BF16),
            pltpu.VMEM((C, C), BF16),
            pltpu.VMEM((C, 128), BF16),
            pltpu.VMEM((C, C), BF16),
            pltpu.VMEM((KC, C), F32),
            pltpu.VMEM((N, NK // N, C), BF16),
            pltpu.VMEM((NK // 2, 128), U32),
            pltpu.VMEM((NC, C // 2, KC), U32),
            pltpu.VMEM((len(FACTORS), C // 4, NK // N), U32),
            pltpu.VMEM((NG, NK, QG), F32),
            pltpu.VMEM((NG, NC, 8, QG), F32),
            pltpu.VMEM((2, len(SLOTS), NK // N, 128), BF16),
            pltpu.VMEM((NG, 8, QG), F32),
            pltpu.VMEM((EG, KC, QG), F32),
            pltpu.VMEM((EG, C, QG), F32),
            pltpu.VMEM((EG + 1, 8, QG), F32),
            pltpu.VMEM((EG, 8, QG), F32),
            pltpu.VMEM((4, ROWS, C, W), BF16),
            pltpu.SemaphoreType.DMA((NC,)),
            pltpu.SemaphoreType.DMA((3,)),
            pltpu.SemaphoreType.DMA((12,)),
        ],
        compiler_params=pltpu.CompilerParams(vmem_limit_bytes=110 * 2**20),
    )(x.reshape(H, W, C).transpose(0, 2, 1), wq, wkv, wo)
    return out.transpose(0, 2, 1).reshape(B, H, W, C)
```
